```python
import jax
import jax.numpy as jnp

def _softmax(x, axis=-1):
    return jax.nn.softmax(x, axis=axis)
def _gelu(x):
    return jax.nn.gelu(x, approximate=True)
def _silu(x):
    return jax.nn.silu(x)
def _sigmoid(x):
    return jax.nn.sigmoid(x)
def _layernorm(x, axis=-1, eps=1e-5):
    m = jnp.mean(x, axis=axis, keepdims=True)
    v = jnp.var(x, axis=axis, keepdims=True)
    return (x - m) / jnp.sqrt(v + eps)
def _scatter_add(tgt, idx, src, axis=0):
    return tgt.at[idx].add(src)
def _segment_sum(src, seg, n):
    return jax.ops.segment_sum(src, seg, n)
class _Rng:
    def __init__(self, key):
        self._k = key
    def _next(self):
        self._k, sub = jax.random.split(self._k)
        return sub
    def normal(self, shape):
        return jax.random.normal(self._next(), shape, dtype=jnp.bfloat16)
    def randint(self, lo, hi, shape):
        return jax.random.randint(self._next(), shape, lo, hi, dtype=jnp.int32)
    def uniform(self, shape, lo=0.0, hi=1.0):
        return jax.random.uniform(self._next(), shape, jnp.bfloat16, lo, hi)
    def permutation(self, n):
        return jax.random.permutation(self._next(), n)


kernel_name = 'sequential_preLN__sliding_block_cached__moe_arch_mod__decode'

def setup_inputs():
    _rng = _Rng(jax.random.key(int.from_bytes(__import__("os").urandom(4), "little")))
    _w = (lambda a: (lambda t: t.astype(jnp.bfloat16) if jnp.issubdtype(t.dtype, jnp.floating) else t)(jnp.asarray(a)))
    def _A_setup():
        B, Sq, D = 1, 1, 640
        Hq, Hkv, Sk, Dh = 32, 32, 32768, 192
        assert Hq % Hkv == 0, (Hq, Hkv)
        return {
            "x": _w((lambda *s: _rng.normal(s) * 0.05)(B, Sq, D)),
            "k_cache": _w((lambda *s: _rng.normal(s) * 0.05)(B, Hkv, Sk, Dh)),
            "v_cache": _w((lambda *s: _rng.normal(s) * 0.05)(B, Hkv, Sk, Dh)),
            "wq": _w((lambda *s: _rng.normal(s) * 0.05)(D, Hq * Dh) * (D ** -0.5)),
            "wo": _w((lambda *s: _rng.normal(s) * 0.05)(Hq * Dh, D) * ((Hq * Dh) ** -0.5)),
        }
    _A_in = _A_setup()

    def _B_setup():
        B, S, D, F, C = 1, 1, 640, 1536, 1
        return {
            "x": _w((lambda *s: _rng.normal(s) * 0.05)(B, S, D)),
            "w_r": _w((lambda *s: _rng.normal(s) * 0.05)(D)),
            "w_gate": _w((lambda *s: _rng.normal(s) * 0.05)(D, F)),
            "w_up": _w((lambda *s: _rng.normal(s) * 0.05)(D, F)),
            "w_down": _w((lambda *s: _rng.normal(s) * 0.05)(F, D)),
        }
    _B_in = _B_setup()

    return {
        "A_x": _A_in["x"],
        "A_k_cache": _A_in["k_cache"],
        "A_v_cache": _A_in["v_cache"],
        "A_wq": _A_in["wq"],
        "A_wo": _A_in["wo"],
        "B_x": _B_in["x"],
        "B_w_r": _B_in["w_r"],
        "B_w_gate": _B_in["w_gate"],
        "B_w_up": _B_in["w_up"],
        "B_w_down": _B_in["w_down"],
    }

def reference(A_x, A_k_cache, A_v_cache, A_wq, A_wo, B_x, B_w_r, B_w_gate, B_w_up, B_w_down):
    def _A_ref(x, k_cache, v_cache, wq, wo):
        B, Sq, D = x.shape
        Hq, Dh = 32, 192
        Hkv, Sk = k_cache.shape[1], k_cache.shape[2]
        W = min(4096, max(256, Sk // 4))
        rep = Hq // Hkv
        q = (lambda x, *d: x.transpose(*d))((x @ wq).reshape(B, Sq, Hq, Dh), 0, 2, 1, 3)
        k = jnp.repeat(k_cache[:, :, Sk - W:, :], rep, axis=1)
        v = jnp.repeat(v_cache[:, :, Sk - W:, :], rep, axis=1)
        scores = jnp.einsum("bhqd,bhkd->bhqk", q, k) * (Dh ** -0.5)
        p = _softmax(scores, axis=-1)
        o = jnp.einsum("bhqk,bhkd->bhqd", p, v)
        return (lambda x, *d: x.transpose(*d))(o, 0, 2, 1, 3).reshape(B, Sq, Hq * Dh) @ wo

    def _B_ref(x, w_r, w_gate, w_up, w_down):
        B, S, D = x.shape
        C = 1
        r = x @ w_r
        idx = jnp.argsort(-r, axis=-1)[:, :C]
        idx_e = jnp.repeat(idx.reshape(B, C, 1), D, axis=2)
        x_sel = jnp.take_along_axis(x, idx_e, axis=1)
        g = _silu(x_sel @ w_gate)
        u = x_sel @ w_up
        y = (g * u) @ w_down
        r_sel = _sigmoid(jnp.take_along_axis(r, idx, axis=1))
        y = y * r_sel.reshape(B, C, 1)
        b_off = (jnp.arange(B) * S).reshape(B, 1)
        flat_idx = (idx + b_off).reshape(B * C)
        zero = (x * 0.0).reshape(B * S, D)
        upd = _scatter_add(zero, flat_idx, y.reshape(B * C, D), axis=0)
        return x + upd.reshape(B, S, D)

    x = A_x
    h = x + _A_ref(_layernorm(x, axis=-1), A_k_cache, A_v_cache, A_wq, A_wo)
    h2 = h + _B_ref(_layernorm(h, axis=-1), B_w_r, B_w_gate, B_w_up, B_w_down)
    return h2
```

```python
import functools

import jax
import jax.numpy as jnp
import jax.experimental.pallas as pl
import jax.experimental.pallas.tpu as pltpu

_HQ = 32
_DH = 192
_G = 2
_NB = 3
_FC = 4
_EPS = 1e-5


def _layernorm(x):
    m = jnp.mean(x, axis=-1, keepdims=True)
    c = x - m
    v = jnp.mean(c * c, axis=-1, keepdims=True)
    return c / jnp.sqrt(v + _EPS)


def _kernel(x_hbm, k_hbm, v_hbm, wq_hbm, wo_hbm, wr_hbm, wg_hbm, wu_hbm, wd_hbm,
            o_ref,
            x_v, wr_v, wq_v, wo_v, wg_v, wu_v, wd_v, k_v, v_v, q_v,
            s_small, s_k, s_v, s_f, *, window):
    f32, bf16 = jnp.float32, jnp.bfloat16
    d_model = x_v.shape[-1]
    seq = k_hbm.shape[-1]
    gr = _G * _DH
    ng = _HQ // _G
    fc = wg_v.shape[-1] // _FC

    def kv_copy(src, dst, sem, g, slot):
        return pltpu.make_async_copy(
            src.at[pl.ds(g * gr, gr), pl.ds(seq - window, window)],
            dst.at[slot], sem.at[slot])

    def ffn_copies(c):
        cs = pl.ds(c * fc, fc)
        return (pltpu.make_async_copy(wg_hbm.at[:, cs], wg_v.at[:, cs], s_f.at[3 * c]),
                pltpu.make_async_copy(wu_hbm.at[:, cs], wu_v.at[:, cs], s_f.at[3 * c + 1]),
                pltpu.make_async_copy(wd_hbm.at[cs, :], wd_v.at[cs, :], s_f.at[3 * c + 2]))

    x_cp = pltpu.make_async_copy(x_hbm, x_v, s_small.at[0])
    wq_cp = pltpu.make_async_copy(wq_hbm, wq_v, s_small.at[1])
    wo_cp = pltpu.make_async_copy(wo_hbm, wo_v, s_small.at[2])
    wr_cp = pltpu.make_async_copy(wr_hbm, wr_v, s_small.at[3])

    x_cp.start()
    wq_cp.start()
    kv_copy(k_hbm, k_v, s_k, 0, 0).start()
    kv_copy(v_hbm, v_v, s_v, 0, 0).start()
    wo_cp.start()
    wr_cp.start()
    for b in range(1, _NB):
        kv_copy(k_hbm, k_v, s_k, b, b).start()
        kv_copy(v_hbm, v_v, s_v, b, b).start()

    x_cp.wait()
    x = x_v[...].astype(f32)
    ln = jnp.broadcast_to(_layernorm(x).astype(bf16), (8, d_model))
    row = jax.lax.broadcasted_iota(jnp.int32, (8, gr), 0)
    col = jax.lax.broadcasted_iota(jnp.int32, (8, gr), 1)
    diag = jnp.logical_and(col >= row * _DH, col < (row + 1) * _DH)
    wq_cp.wait()
    for g in range(ng):
        q = jnp.dot(ln, wq_v[:, g * gr:(g + 1) * gr], preferred_element_type=f32)
        q_v[g] = jnp.where(diag, q, 0.0)

    scale = _DH ** -0.5

    def body(g, acc):
        slot = g % _NB
        kv_copy(k_hbm, k_v, s_k, g, slot).wait()
        s = jnp.dot(q_v[g].astype(bf16), k_v[slot], preferred_element_type=f32) * scale

        @pl.when(g + _NB < ng)
        def _():
            kv_copy(k_hbm, k_v, s_k, g + _NB, slot).start()

        @pl.when(g == ng - 1)
        def _():
            for c in range(_FC):
                for cp in ffn_copies(c):
                    cp.start()

        m = jnp.max(s, axis=-1, keepdims=True)
        p = jnp.exp(s - m)
        l = jnp.sum(p, axis=-1, keepdims=True)
        kv_copy(v_hbm, v_v, s_v, g, slot).wait()
        r = jax.lax.dot_general(p.astype(bf16), v_v[slot], (((1,), (1,)), ((), ())),
                                preferred_element_type=f32)

        @pl.when(g + _NB < ng)
        def _():
            kv_copy(v_hbm, v_v, s_v, g + _NB, slot).start()

        @pl.when(g == 0)
        def _():
            wo_cp.wait()

        o = jnp.where(diag, r / l, 0.0).astype(bf16)
        w = wo_v[pl.ds(pl.multiple_of(g * gr, gr), gr), :]
        return acc + jnp.dot(o, w, preferred_element_type=f32)

    acc = jax.lax.fori_loop(0, ng, body, jnp.zeros((8, d_model), f32))
    h = x + jnp.sum(acc, axis=0, keepdims=True)
    ln2 = _layernorm(h)
    ln2b = ln2.astype(bf16)
    wr_cp.wait()
    r = jnp.sum(ln2b.astype(f32) * wr_v[...].astype(f32), axis=-1, keepdims=True)
    gate = jax.nn.sigmoid(r)
    lhs = jnp.broadcast_to(ln2b, (8, d_model))
    y = jnp.zeros((8, d_model), f32)
    for c in range(_FC):
        cg, cu, cd = ffn_copies(c)
        cs = slice(c * fc, (c + 1) * fc)
        cg.wait()
        a = jnp.dot(lhs, wg_v[:, cs], preferred_element_type=f32)
        cu.wait()
        u = jnp.dot(lhs, wu_v[:, cs], preferred_element_type=f32)
        t = (a * jax.nn.sigmoid(a) * u).astype(bf16)
        cd.wait()
        y = y + jnp.dot(t, wd_v[cs, :], preferred_element_type=f32)
    o_ref[...] = (h + (ln2 + y[0:1] * gate)).astype(o_ref.dtype)


@jax.jit
def pallas_sequential_preLN__sliding_block_cached__moe_arch_mod__decode_kernel(
    A_x: jax.Array,
    A_k_cache: jax.Array,
    A_v_cache: jax.Array,
    A_wq: jax.Array,
    A_wo: jax.Array,
    B_x: jax.Array,
    B_w_r: jax.Array,
    B_w_gate: jax.Array,
    B_w_up: jax.Array,
    B_w_down: jax.Array,
):
    del B_x
    _, _, d_model = A_x.shape
    _, hkv, seq, dh = A_k_cache.shape
    assert (hkv, dh) == (_HQ, _DH) and A_x.shape[:2] == (1, 1)
    window = min(4096, max(256, seq // 4))
    ffn = B_w_gate.shape[1]
    dt = A_x.dtype

    x = A_x.reshape(1, d_model)
    k = A_k_cache.transpose(0, 1, 3, 2).reshape(hkv * dh, seq)
    v = A_v_cache.transpose(0, 1, 3, 2).reshape(hkv * dh, seq)
    wr = B_w_r.reshape(1, d_model)

    gr = _G * _DH
    hbm = pl.BlockSpec(memory_space=pltpu.HBM)
    out = pl.pallas_call(
        functools.partial(_kernel, window=window),
        in_specs=[hbm] * 9,
        out_specs=pl.BlockSpec(memory_space=pltpu.VMEM),
        out_shape=jax.ShapeDtypeStruct((1, d_model), dt),
        scratch_shapes=[
            pltpu.VMEM((1, d_model), dt),
            pltpu.VMEM((1, d_model), dt),
            pltpu.VMEM(A_wq.shape, dt),
            pltpu.VMEM(A_wo.shape, dt),
            pltpu.VMEM((d_model, ffn), dt),
            pltpu.VMEM((d_model, ffn), dt),
            pltpu.VMEM((ffn, d_model), dt),
            pltpu.VMEM((_NB, gr, window), dt),
            pltpu.VMEM((_NB, gr, window), dt),
            pltpu.VMEM((_HQ // _G, 8, gr), jnp.float32),
            pltpu.SemaphoreType.DMA((4,)),
            pltpu.SemaphoreType.DMA((_NB,)),
            pltpu.SemaphoreType.DMA((_NB,)),
            pltpu.SemaphoreType.DMA((3 * _FC,)),
        ],
        compiler_params=pltpu.CompilerParams(vmem_limit_bytes=100 * 1024 * 1024),
    )(x, k, v, A_wq, A_wo, wr, B_w_gate, B_w_up, B_w_down)
    return out.reshape(A_x.shape)
```

```python
import functools

import jax
import jax.numpy as jnp
import jax.experimental.pallas as pl
import jax.experimental.pallas.tpu as pltpu

_HQ = 32
_DH = 192
_G = 2
_NB = 2
_DC = (4, 4, 3, 1)
_EPS = 1e-5


def _layernorm(x):
    m = jnp.mean(x, axis=-1, keepdims=True)
    c = x - m
    v = jnp.mean(c * c, axis=-1, keepdims=True)
    return c / jnp.sqrt(v + _EPS)


def _kernel(x_hbm, k_hbm, v_hbm, wq_hbm, wo_hbm, wr_hbm, wg_hbm, wu_hbm, wd_hbm,
            o_ref,
            x_v, wr_v, wq_v, wo_v, wg_v, wu_v, wd_v, k_v, v_v, q_v,
            s_small, s_k, s_v, s_f, *, window):
    f32, bf16 = jnp.float32, jnp.bfloat16
    d_model = x_v.shape[-1]
    seq = k_hbm.shape[-1]
    gr = _G * _DH
    ng = _HQ // _G
    fc = wg_v.shape[-1] // sum(_DC)

    def kv_copy(src, dst, sem, g, slot):
        return pltpu.make_async_copy(
            src.at[pl.ds(g * gr, gr), pl.ds(seq - window, window)],
            dst.at[slot], sem.at[slot])

    wg_cp = pltpu.make_async_copy(wg_hbm, wg_v, s_f.at[0])
    wu_cp = pltpu.make_async_copy(wu_hbm, wu_v, s_f.at[1])
    wd_rows = [slice(sum(_DC[:c]) * fc, sum(_DC[:c + 1]) * fc) for c in range(len(_DC))]
    wd_cps = [pltpu.make_async_copy(wd_hbm.at[rs, :], wd_v.at[rs, :], s_f.at[2 + c])
              for c, rs in enumerate(wd_rows)]

    x_cp = pltpu.make_async_copy(x_hbm, x_v, s_small.at[0])
    wq_cp = pltpu.make_async_copy(wq_hbm, wq_v, s_small.at[1])
    wo_cp = pltpu.make_async_copy(wo_hbm, wo_v, s_small.at[2])
    wr_cp = pltpu.make_async_copy(wr_hbm, wr_v, s_small.at[3])

    x_cp.start()
    wq_cp.start()
    kv_copy(k_hbm, k_v, s_k, 0, 0).start()
    kv_copy(v_hbm, v_v, s_v, 0, 0).start()
    wo_cp.start()
    wr_cp.start()
    for b in range(1, _NB):
        kv_copy(k_hbm, k_v, s_k, b, b).start()
        kv_copy(v_hbm, v_v, s_v, b, b).start()

    x_cp.wait()
    x = x_v[...].astype(f32)
    ln = jnp.broadcast_to(_layernorm(x).astype(bf16), (8, d_model))
    row = jax.lax.broadcasted_iota(jnp.int32, (8, gr), 0)
    col = jax.lax.broadcasted_iota(jnp.int32, (8, gr), 1)
    diag = jnp.logical_and(col >= row * _DH, col < (row + 1) * _DH)
    wq_cp.wait()
    for g in range(ng):
        q = jnp.dot(ln, wq_v[:, g * gr:(g + 1) * gr], preferred_element_type=f32)
        q_v[g] = jnp.where(diag, q, 0.0)

    scale = _DH ** -0.5

    def body(g, acc):
        slot = g % _NB
        kv_copy(k_hbm, k_v, s_k, g, slot).wait()
        s = jnp.dot(q_v[g].astype(bf16), k_v[slot], preferred_element_type=f32) * scale

        @pl.when(g + _NB < ng)
        def _():
            kv_copy(k_hbm, k_v, s_k, g + _NB, slot).start()

        @pl.when(g == ng - 1)
        def _():
            for cp in (wg_cp, wu_cp, *wd_cps):
                cp.start()

        m = jnp.max(s, axis=-1, keepdims=True)
        p = jnp.exp(s - m)
        l = jnp.sum(p, axis=-1, keepdims=True)
        kv_copy(v_hbm, v_v, s_v, g, slot).wait()
        r = jax.lax.dot_general(p.astype(bf16), v_v[slot], (((1,), (1,)), ((), ())),
                                preferred_element_type=f32)

        @pl.when(g + _NB < ng)
        def _():
            kv_copy(v_hbm, v_v, s_v, g + _NB, slot).start()

        @pl.when(g == 0)
        def _():
            wo_cp.wait()

        o = jnp.where(diag, r / l, 0.0).astype(bf16)
        w = wo_v[pl.ds(pl.multiple_of(g * gr, gr), gr), :]
        return acc + jnp.dot(o, w, preferred_element_type=f32)

    acc = jax.lax.fori_loop(0, ng, body, jnp.zeros((8, d_model), f32))
    h = x + jnp.sum(acc, axis=0, keepdims=True)
    ln2 = _layernorm(h)
    ln2b = ln2.astype(bf16)
    wr_cp.wait()
    r = jnp.sum(ln2b.astype(f32) * wr_v[...].astype(f32).reshape(1, d_model), axis=-1, keepdims=True)
    gate = jax.nn.sigmoid(r)
    lhs = jnp.broadcast_to(ln2b, (8, d_model))
    wg_cp.wait()
    a = jnp.dot(lhs, wg_v[...], preferred_element_type=f32)
    wu_cp.wait()
    u = jnp.dot(lhs, wu_v[...], preferred_element_type=f32)
    t = (a * jax.nn.sigmoid(a) * u).astype(bf16)
    y = jnp.zeros((8, d_model), f32)
    for rs, cp in zip(wd_rows, wd_cps):
        cp.wait()
        y = y + jnp.dot(t[:, rs], wd_v[rs, :], preferred_element_type=f32)
    o_ref[...] = (h + (ln2 + y[0:1] * gate)).astype(o_ref.dtype)


@jax.jit
def pallas_sequential_preLN__sliding_block_cached__moe_arch_mod__decode_kernel(
    A_x: jax.Array,
    A_k_cache: jax.Array,
    A_v_cache: jax.Array,
    A_wq: jax.Array,
    A_wo: jax.Array,
    B_x: jax.Array,
    B_w_r: jax.Array,
    B_w_gate: jax.Array,
    B_w_up: jax.Array,
    B_w_down: jax.Array,
):
    del B_x
    _, _, d_model = A_x.shape
    _, hkv, seq, dh = A_k_cache.shape
    assert (hkv, dh) == (_HQ, _DH) and A_x.shape[:2] == (1, 1)
    window = min(4096, max(256, seq // 4))
    ffn = B_w_gate.shape[1]
    dt = A_x.dtype

    x = A_x.reshape(1, d_model)
    k = A_k_cache.transpose(0, 1, 3, 2).reshape(hkv * dh, seq)
    v = A_v_cache.transpose(0, 1, 3, 2).reshape(hkv * dh, seq)

    gr = _G * _DH
    hbm = pl.BlockSpec(memory_space=pltpu.HBM)
    out = pl.pallas_call(
        functools.partial(_kernel, window=window),
        in_specs=[hbm] * 9,
        out_specs=pl.BlockSpec(memory_space=pltpu.VMEM),
        out_shape=jax.ShapeDtypeStruct((1, d_model), dt),
        scratch_shapes=[
            pltpu.VMEM((1, d_model), dt),
            pltpu.VMEM((d_model,), dt),
            pltpu.VMEM(A_wq.shape, dt),
            pltpu.VMEM(A_wo.shape, dt),
            pltpu.VMEM((d_model, ffn), dt),
            pltpu.VMEM((d_model, ffn), dt),
            pltpu.VMEM((ffn, d_model), dt),
            pltpu.VMEM((_NB, gr, window), dt),
            pltpu.VMEM((_NB, gr, window), dt),
            pltpu.VMEM((_HQ // _G, 8, gr), jnp.float32),
            pltpu.SemaphoreType.DMA((4,)),
            pltpu.SemaphoreType.DMA((_NB,)),
            pltpu.SemaphoreType.DMA((_NB,)),
            pltpu.SemaphoreType.DMA((2 + len(_DC),)),
        ],
        compiler_params=pltpu.CompilerParams(vmem_limit_bytes=100 * 1024 * 1024),
    )(x, k, v, A_wq, A_wo, B_w_r, B_w_gate, B_w_up, B_w_down)
    return out.reshape(A_x.shape)
```
